```python
import os as _os
_os.environ.setdefault("JAX_PLATFORMS", "cpu")
import jax
import jax.numpy as jnp

def _softmax(x, axis=-1):
    return jax.nn.softmax(x, axis=axis)
def _gelu(x):
    return jax.nn.gelu(x, approximate=True)
def _silu(x):
    return jax.nn.silu(x)
def _sigmoid(x):
    return jax.nn.sigmoid(x)
def _layernorm(x, axis=-1, eps=1e-5):
    m = jnp.mean(x, axis=axis, keepdims=True)
    v = jnp.var(x, axis=axis, keepdims=True)
    return (x - m) / jnp.sqrt(v + eps)
def _scatter_add(tgt, idx, src, axis=0):
    return tgt.at[idx].add(src)
def _segment_sum(src, seg, n):
    return jax.ops.segment_sum(src, seg, n)
class _Rng:
    def __init__(self, key):
        self._k = key
    def _next(self):
        self._k, sub = jax.random.split(self._k)
        return sub
    def normal(self, shape):
        return jax.random.normal(self._next(), shape, dtype=jnp.bfloat16)
    def randint(self, lo, hi, shape):
        return jax.random.randint(self._next(), shape, lo, hi, dtype=jnp.int32)
    def uniform(self, shape, lo=0.0, hi=1.0):
        return jax.random.uniform(self._next(), shape, jnp.bfloat16, lo, hi)
    def permutation(self, n):
        return jax.random.permutation(self._next(), n)


kernel_name = 'concat_heads__gqa_block_cached__mha_block_cached__near_ridge'

def setup_inputs():
    _rng = _Rng(jax.random.key(int.from_bytes(__import__("os").urandom(4), "little")))
    _w = (lambda a: (lambda t: t.astype(jnp.bfloat16) if jnp.issubdtype(t.dtype, jnp.floating) else t)(jnp.asarray(a)))
    def _A_setup():
        B, Sq, D = 8, 48, 512
        Hq, Hkv, Sk, Dh = 32, 8, 1024, 128
        assert Hq % Hkv == 0, (Hq, Hkv)
        return {
            "x": _w((lambda *s: _rng.normal(s) * 0.8)(B, Sq, D)),
            "k_cache": _w((lambda *s: _rng.normal(s) * 0.8)(B, Hkv, Sk, Dh)),
            "v_cache": _w((lambda *s: _rng.normal(s) * 0.05)(B, Hkv, Sk, Dh)),
            "wq": _w((lambda *s: _rng.normal(s) * 0.8)(D, Hq * Dh) * (D ** -0.5)),
            "wo": _w((lambda *s: _rng.normal(s) * 0.05)(Hq * Dh, D) * ((Hq * Dh) ** -0.5)),
        }
    _A_in = _A_setup()

    def _B_setup():
        B, Sq, D = 8, 48, 512
        H, Sk, Dh = 32, 1024, 128
        return {
            "x": _w((lambda *s: _rng.normal(s) * 0.8)(B, Sq, D)),
            "k_cache": _w((lambda *s: _rng.normal(s) * 0.8)(B, H, Sk, Dh)),
            "v_cache": _w((lambda *s: _rng.normal(s) * 0.05)(B, H, Sk, Dh)),
            "wq": _w((lambda *s: _rng.normal(s) * 0.8)(D, H * Dh) * (D ** -0.5)),
            "wo": _w((lambda *s: _rng.normal(s) * 0.05)(H * Dh, D) * ((H * Dh) ** -0.5)),
        }
    _B_in = _B_setup()

    return {
        "A_x": _A_in["x"],
        "A_k_cache": _A_in["k_cache"],
        "A_v_cache": _A_in["v_cache"],
        "A_wq": _A_in["wq"],
        "A_wo": _A_in["wo"],
        "B_x": _B_in["x"],
        "B_k_cache": _B_in["k_cache"],
        "B_v_cache": _B_in["v_cache"],
        "B_wq": _B_in["wq"],
        "B_wo": _B_in["wo"],
    }

def reference(A_x, A_k_cache, A_v_cache, A_wq, A_wo, B_x, B_k_cache, B_v_cache, B_wq, B_wo):
    def _A_ref(x, k_cache, v_cache, wq, wo):
        B, Sq, D = x.shape
        Hq, Dh = 32, 128
        Hkv = k_cache.shape[1]
        rep = Hq // Hkv
        q = (lambda x, *d: x.transpose(*d))((x @ wq).reshape(B, Sq, Hq, Dh), 0, 2, 1, 3)
        k = jnp.repeat(k_cache, rep, axis=1)
        v = jnp.repeat(v_cache, rep, axis=1)
        scores = jnp.einsum("bhqd,bhkd->bhqk", q, k) * (Dh ** -0.5)
        p = _softmax(scores, axis=-1)
        o = jnp.einsum("bhqk,bhkd->bhqd", p, v)
        return (lambda x, *d: x.transpose(*d))(o, 0, 2, 1, 3).reshape(B, Sq, Hq * Dh) @ wo

    def _B_ref(x, k_cache, v_cache, wq, wo):
        B, Sq, D = x.shape
        H, Dh = 32, 128
        q = (lambda x, *d: x.transpose(*d))((x @ wq).reshape(B, Sq, H, Dh), 0, 2, 1, 3)
        scores = jnp.einsum("bhqd,bhkd->bhqk", q, k_cache) * (Dh ** -0.5)
        p = _softmax(scores, axis=-1)
        o = jnp.einsum("bhqk,bhkd->bhqd", p, v_cache)
        return (lambda x, *d: x.transpose(*d))(o, 0, 2, 1, 3).reshape(B, Sq, H * Dh) @ wo

    a = _A_ref(A_x, A_k_cache, A_v_cache, A_wq, A_wo)
    b = _B_ref(B_x, B_k_cache, B_v_cache, B_wq, B_wo)
    return jnp.concatenate([a, b], axis=-1)
```

```python
import functools
import jax
import jax.numpy as jnp
import numpy as np
from jax import lax
from jax.experimental import pallas as pl
from jax.experimental.pallas import tpu as pltpu

B, SQ, D = 8, 48, 512
HQ, HKV, SK, DH = 32, 8, 1024, 128
REP = HQ // HKV
M = B * SQ
GW = REP * DH
QSCALE = float(DH ** -0.5 * np.log2(np.e))
CPR = 16
PR = SK // CPR
NPAIR = B // 2


def _build(name="concat_heads_attention", shift=2, sched=None, do_dma=True, do_compute=True,
         semchk=False, bchk=False, flags=None, vmem_mb=64, skipq=True):
    if sched is None:
        sched = (2, 1, 2, 2, 2, 2, 1, 1, 1, 1, 1, 1, 1, 2)
    assert sum(sched) == CPR + 4 and len(sched) == 14

    def kernel(xa_hbm, ka_hbm, va_hbm, wqa_hbm, woa_hbm, xb_hbm, kb_hbm, vb_hbm, wqb_hbm, wob_hbm,
               out_hbm, x_buf, wq_buf, wo_buf, kva_buf, kvb_buf, qa_buf, qb_buf, acc, out_buf,
               w_sem, a_sem, b_sem, out_sem):

        def start_a(g, c):
            slot = g & 1
            rows = pl.ds(pl.multiple_of(c * PR, PR), PR)
            for d in range(NPAIR):
                bs = pl.ds(2 * d, 2)
                for a, src in enumerate((ka_hbm, va_hbm)):
                    pltpu.make_async_copy(src.at[bs, g, rows], kva_buf.at[slot, d, a, :, rows],
                                          a_sem.at[slot]).start(priority=a)

        def start_b(h, c):
            slot = h & 1
            last = h == HQ - 1
            for d in range(NPAIR):
                if isinstance(h, int):
                    p, piece = (c // 4, 4 * (c % 4) + d) if last else (d, c)
                else:
                    p = jnp.where(last, c // 4, d)
                    piece = jnp.where(last, 4 * (c % 4) + d, c)
                rows = pl.ds(pl.multiple_of(piece * PR, PR), PR)
                bs = pl.ds(2 * p, 2)
                for a, src in enumerate((kb_hbm, vb_hbm)):
                    pltpu.make_async_copy(src.at[bs, h, rows], kvb_buf.at[slot, p, a, :, rows],
                                          b_sem.at[slot * NPAIR + p]).start(priority=a)

        def load(ref):
            return pltpu.bitcast(ref.bitcast(jnp.uint32)[...], jnp.bfloat16)

        def scores(q, k):
            return lax.dot_general(q, k, (((1,), (1,)), ((), ())), preferred_element_type=jnp.float32)

        def weighted(s, v):
            m = jnp.max(s, axis=1, keepdims=True)
            p = jnp.exp2(s - m)
            l = jnp.sum(p, axis=1, keepdims=True)
            o = jnp.dot(p.astype(jnp.bfloat16), v, preferred_element_type=jnp.float32)
            return o * (1.0 / l)

        def project_q(t, h):
            w = wq_buf[t, :, :, pl.ds(pl.multiple_of(h * DH, DH), DH)].reshape(D, DH)
            q = jnp.dot(x_buf[t], w, preferred_element_type=jnp.float32)
            return pltpu.bitcast((q * QSCALE).astype(jnp.bfloat16), jnp.uint32)

        if do_dma:
            pltpu.make_async_copy(xa_hbm, x_buf.at[0], w_sem.at[0]).start(priority=0)
            pltpu.make_async_copy(xb_hbm, x_buf.at[1], w_sem.at[0]).start(priority=1)

            def w_body(i, _):
                rq = pl.ds(pl.multiple_of((i >> 2) * 8, 8), 8)
                cq = pl.ds(pl.multiple_of((i & 3) * 1024, 1024), 1024)
                ro = pl.ds(pl.multiple_of(i * 16, 16), 16)
                for d in range(2):
                    ss = pl.ds(2 * d, 2)
                    for t, src in enumerate((wqa_hbm, wqb_hbm)):
                        pltpu.make_async_copy(src.at[ss, rq, cq], wq_buf.at[t, ss, rq, cq], w_sem.at[1]).start(priority=t)
                for d in range(2):
                    ss = pl.ds(2 * d, 2)
                    for t, src in enumerate((woa_hbm, wob_hbm)):
                        pltpu.make_async_copy(src.at[ss, ro], wo_buf.at[t, ss, ro], w_sem.at[2]).start(priority=t)
            lax.fori_loop(0, 64, w_body, None)
            lax.fori_loop(0, CPR, lambda c, _: start_a(0, c), None)
        acc[...] = jnp.zeros_like(acc)
        if do_dma:
            pltpu.make_async_copy(x_buf, x_buf, w_sem.at[0]).wait()
            pltpu.make_async_copy(wq_buf, wq_buf, w_sem.at[1]).wait()
            pltpu.make_async_copy(wo_buf, wo_buf, w_sem.at[2]).wait()

        n0 = CPR - shift
        def q0_body(j, _):
            if do_dma:
                lax.fori_loop(n0 * j // REP, n0 * (j + 1) // REP, lambda c, _: start_b(0, c), None)
            if do_compute:
                qa_buf[0, j] = project_q(0, j)
        lax.fori_loop(0, REP, q0_body, None)
        if do_compute:
            qb_buf[0] = project_q(1, 0)

        def body(n, _):
            g, quarter = n >> 2, n & 3
            todo = [("b", 0, c) for c in range(CPR - shift, CPR)] + [("a", 0, c) for c in range(4)] \
                + [("b", 1, c) for c in range(CPR - shift)]
            points = iter(sched)

            def issue():
                cnt = next(points)
                mine = [todo.pop(0) for _ in range(cnt)]
                if not do_dma:
                    return
                for kind, ahead, c in mine:
                    if kind == "a":
                        @pl.when(g + 1 < HKV)
                        def _():
                            start_a(g + 1, quarter * 4 + c)
                    elif ahead:
                        @pl.when(n + 1 < HQ)
                        def _():
                            start_b(n + 1, c)
                    else:
                        start_b(n, c)

            def maybe(f):
                if skipq:
                    pl.when(n + 1 < HQ)(f)
                else:
                    f()

            issue()
            if do_compute:
                @maybe
                def _():
                    qb_buf[(n + 1) & 1] = project_q(1, jnp.minimum(n + 1, HQ - 1))
            issue()
            if do_compute:
                @maybe
                def _():
                    qa_buf[(g + 1) & 1, quarter] = project_q(0, jnp.minimum(n + REP, HQ - 1))

            if do_dma:
                @pl.when(quarter == 0)
                def _():
                    dst = kva_buf.at[g & 1]
                    pltpu.make_async_copy(dst, dst, a_sem.at[g & 1]).wait()

            oa = []
            for i in range(2):
                issue()
                if do_compute:
                    r0 = pl.multiple_of((2 * quarter + i) * (SQ // 2), SQ // 2)
                    q = qa_buf[g & 1, :, pl.ds(r0, SQ // 2)].reshape(REP * SQ // 2, DH)
                    s = scores(pltpu.bitcast(q, jnp.bfloat16), load(kva_buf.at[g & 1, quarter, 0, i]))
                issue()
                if do_compute:
                    o = weighted(s, load(kva_buf.at[g & 1, quarter, 1, i]))
                    oa.append(jnp.concatenate([o[j * SQ:(j + 1) * SQ] for j in range(REP)], axis=1))
            rows_a = pl.ds(pl.multiple_of(quarter * 2 * SQ, 2 * SQ), 2 * SQ)

            def out_a():
                w = wo_buf[0, g >> 1, pl.ds(pl.multiple_of((g & 1) * GW, GW), GW)]
                acc[0, rows_a] += jnp.dot(jnp.concatenate(oa, axis=0).astype(jnp.bfloat16), w,
                                          preferred_element_type=jnp.float32)

            def finish(t, rows, cond):
                @pl.when(cond)
                def _():
                    out_buf[t, rows] = acc[t, rows].astype(jnp.bfloat16)
                    pltpu.make_async_copy(out_buf.at[t, rows], out_hbm.at[rows, pl.ds(t * D, D)], out_sem).start()

            slot = n & 1

            def qk(b):
                if b % 2 == 0 and do_dma:
                    dst = kvb_buf.at[slot, b // 2]
                    pltpu.make_async_copy(dst, dst, b_sem.at[slot * NPAIR + b // 2]).wait()
                if do_compute:
                    q = pltpu.bitcast(qb_buf[slot, pl.ds(b * SQ // 2, SQ // 2)], jnp.bfloat16)
                    return scores(q, load(kvb_buf.at[slot, b // 2, 0, b % 2]))

            def out_b(p):
                rows = pl.ds(p * 2 * SQ, 2 * SQ)
                if do_compute:
                    w = wo_buf[1, n >> 3, pl.ds(pl.multiple_of((n & 7) * DH, DH), DH)]
                    o = jnp.concatenate(ob[2 * p:2 * p + 2], axis=0).astype(jnp.bfloat16)
                    acc[1, rows] += jnp.dot(o, w, preferred_element_type=jnp.float32)
                finish(1, rows, n == HQ - 1)

            sb = [qk(0)]
            if do_compute:
                out_a()
            finish(0, rows_a, g == HKV - 1)
            ob = []
            for b in range(B):
                issue()
                if b + 1 < B:
                    sb.append(qk(b + 1))
                if do_compute:
                    ob.append(weighted(sb[b], load(kvb_buf.at[slot, b // 2, 1, b % 2])))
                if b % 2 == 0 and b >= 2:
                    out_b(b // 2 - 1)
            out_b(NPAIR - 1)

        lax.fori_loop(0, HQ, body, None)
        pltpu.make_async_copy(out_buf, out_buf, out_sem).wait()

    def f(A_x, A_k_cache, A_v_cache, A_wq, A_wo, B_x, B_k_cache, B_v_cache, B_wq, B_wo):
        out = pl.pallas_call(
            kernel, name=name,
            in_specs=[pl.BlockSpec(memory_space=pl.ANY)] * 10,
            out_specs=pl.BlockSpec(memory_space=pl.ANY),
            out_shape=jax.ShapeDtypeStruct((M, 2 * D), jnp.bfloat16),
            scratch_shapes=[
                pltpu.VMEM((2, M, D), jnp.bfloat16),
                pltpu.VMEM((2, 4, D // 4, HQ * DH), jnp.bfloat16),
                pltpu.VMEM((2, 4, HQ * DH // 4, D), jnp.bfloat16),
                pltpu.VMEM((2, NPAIR, 2, 2, SK, DH), jnp.bfloat16),
                pltpu.VMEM((2, NPAIR, 2, 2, SK, DH), jnp.bfloat16),
                pltpu.VMEM((2, REP, M // 2, DH), jnp.uint32),
                pltpu.VMEM((2, M // 2, DH), jnp.uint32),
                pltpu.VMEM((2, M, D), jnp.float32),
                pltpu.VMEM((2, M, D), jnp.bfloat16),
                pltpu.SemaphoreType.DMA((3,)),
                pltpu.SemaphoreType.DMA((2,)),
                pltpu.SemaphoreType.DMA((2 * NPAIR,)),
                pltpu.SemaphoreType.DMA(()),
            ],
            compiler_params=pltpu.CompilerParams(
                vmem_limit_bytes=vmem_mb * 2**20, disable_bounds_checks=not bchk,
                disable_semaphore_checks=not semchk, flags=flags),
        )(A_x.reshape(M, D), A_k_cache, A_v_cache, A_wq.reshape(4, D // 4, HQ * DH), A_wo.reshape(4, HQ * DH // 4, D),
          B_x.reshape(M, D), B_k_cache, B_v_cache, B_wq.reshape(4, D // 4, HQ * DH), B_wo.reshape(4, HQ * DH // 4, D))
        return out.reshape(B, SQ, 2 * D)
    return f


@jax.jit
def pallas_concat_heads__gqa_block_cached__mha_block_cached__near_ridge_kernel(
    A_x, A_k_cache, A_v_cache, A_wq, A_wo, B_x, B_k_cache, B_v_cache, B_wq, B_wo,
):
    return _build()(A_x, A_k_cache, A_v_cache, A_wq, A_wo, B_x, B_k_cache, B_v_cache, B_wq, B_wo)
```

```python
import functools
import jax
import jax.numpy as jnp
import numpy as np
from jax import lax
from jax.experimental import pallas as pl
from jax.experimental.pallas import tpu as pltpu

B, SQ, D = 8, 48, 512
HQ, HKV, SK, DH = 32, 8, 1024, 128
REP = HQ // HKV
M = B * SQ
GW = REP * DH
QSCALE = float(DH ** -0.5 * np.log2(np.e))
CPR = 16
PR = SK // CPR
NPAIR = B // 2


def _build(name="concat_heads_attention", sched1=(2, 2, 2, 2, 2, 2), sched2=(1, 1, 1, 1, 1, 1, 1, 1), do_dma=True, do_compute=True,
         semchk=False, bchk=False, flags=None, vmem_mb=64, defer=True, wmode=0, xmode=1, oprio=(0, 1, 0),
         osplit=1, lastseq=True, apos=12, ahead=1, send1="v2", early23=True):
    assert sum(sched1) + sum(sched2) == CPR + 4
    assert ahead == 0 or apos >= sum(sched1)

    def kernel(xa_hbm, ka_hbm, va_hbm, wqa_hbm, woa_hbm, xb_hbm, kb_hbm, vb_hbm, wqb_hbm, wob_hbm,
               out_hbm, x_buf, wq_buf, wo_buf, kva_buf, kvb_buf, qa_buf, qb_buf, acc, out_buf,
               w_sem, a_sem, b_sem, out_sem):

        def start_a(g, c):
            slot = g & 1
            rows = pl.ds(pl.multiple_of(c * PR, PR), PR)
            for d in range(NPAIR):
                bs = pl.ds(2 * d, 2)
                for a, src in enumerate((ka_hbm, va_hbm)):
                    pltpu.make_async_copy(src.at[bs, g, rows], kva_buf.at[slot, d, a, :, rows],
                                          a_sem.at[slot]).start(priority=a)

        def start_b(h, c):
            slot = h & 1
            last = h == HQ - 1
            for d in range(NPAIR):
                if not lastseq:
                    p, piece = d, c
                elif isinstance(h, int):
                    p, piece = (c // 4, 4 * (c % 4) + d) if last else (d, c)
                else:
                    p = jnp.where(last, c // 4, d)
                    piece = jnp.where(last, 4 * (c % 4) + d, c)
                rows = pl.ds(pl.multiple_of(piece * PR, PR), PR)
                bs = pl.ds(2 * p, 2)
                for a, src in enumerate((kb_hbm, vb_hbm)):
                    pltpu.make_async_copy(src.at[bs, h, rows], kvb_buf.at[slot, p, a, :, rows],
                                          b_sem.at[(slot * NPAIR + p) * 2 + a]).start(priority=a)

        def load(ref):
            return pltpu.bitcast(ref.bitcast(jnp.uint32)[...], jnp.bfloat16)

        def scores(q, k):
            return lax.dot_general(q, k, (((1,), (1,)), ((), ())), preferred_element_type=jnp.float32)

        def softmax(s):
            m = jnp.max(s, axis=1, keepdims=True)
            p = jnp.exp2(s - m)
            l = jnp.sum(p, axis=1, keepdims=True)
            return p.astype(jnp.bfloat16), 1.0 / l

        def weighted(pr, v):
            p, r = pr
            return jnp.dot(p, v, preferred_element_type=jnp.float32) * r

        def project_q(t, h):
            w = wq_buf[t, :, :, pl.ds(pl.multiple_of(h * DH, DH), DH)].reshape(D, DH)
            q = jnp.dot(x_buf[t], w, preferred_element_type=jnp.float32)
            return pltpu.bitcast((q * QSCALE).astype(jnp.bfloat16), jnp.uint32)

        if do_dma:
            def start_x():
                if xmode == 0:
                    pltpu.make_async_copy(xa_hbm, x_buf.at[0], w_sem.at[0]).start(priority=0)
                    pltpu.make_async_copy(xb_hbm, x_buf.at[1], w_sem.at[0]).start(priority=1)
                else:
                    for r in range(0, M, 32):
                        for t, src in enumerate((xa_hbm, xb_hbm)):
                            pltpu.make_async_copy(src.at[pl.ds(r, 32)], x_buf.at[t, pl.ds(r, 32)], w_sem.at[0]).start(priority=t)
            start_x()

            def w_body(i, _):
                rq = pl.ds(pl.multiple_of((i >> 2) * 8, 8), 8)
                cq = pl.ds(pl.multiple_of((i & 3) * 1024, 1024), 1024)
                ro = pl.ds(pl.multiple_of(i * 16, 16), 16)
                def wq(d, t):
                    ss = pl.ds(2 * d, 2)
                    src = (wqa_hbm, wqb_hbm)[t]
                    return pltpu.make_async_copy(src.at[ss, rq, cq], wq_buf.at[t, ss, rq, cq], w_sem.at[1])
                def wo(d, t):
                    ss = pl.ds(2 * d, 2)
                    src = (woa_hbm, wob_hbm)[t]
                    return pltpu.make_async_copy(src.at[ss, ro], wo_buf.at[t, ss, ro], w_sem.at[2])
                if wmode == 0:
                    lst = [wq(0, 0), wq(0, 1), wq(1, 0), wq(1, 1), wo(0, 0), wo(0, 1), wo(1, 0), wo(1, 1)]
                elif wmode == 1:
                    lst = [wq(0, 0), wq(0, 1), wo(0, 0), wo(0, 1), wq(1, 0), wq(1, 1), wo(1, 0), wo(1, 1)]
                elif wmode == 2:
                    lst = [wq(0, 0), wo(0, 0), wq(1, 0), wo(1, 0), wq(0, 1), wo(0, 1), wq(1, 1), wo(1, 1)]
                elif wmode == 3:
                    lst = [wq(0, 0), wq(0, 1), wq(1, 0), wq(1, 1)]
                elif wmode == 4:
                    lst = [wo(0, 0), wo(0, 1), wo(1, 0), wo(1, 1)]
                for j, c in enumerate(lst):
                    c.start(priority=j % 2)
            lax.fori_loop(0, 64, w_body, None)
            if wmode == 3:
                def w_body2(i, _):
                    ro = pl.ds(pl.multiple_of(i * 16, 16), 16)
                    for d in range(2):
                        ss = pl.ds(2 * d, 2)
                        for t, src in enumerate((woa_hbm, wob_hbm)):
                            pltpu.make_async_copy(src.at[ss, ro], wo_buf.at[t, ss, ro], w_sem.at[2]).start(priority=t)
                lax.fori_loop(0, 64, w_body2, None)
            lax.fori_loop(0, CPR + 4 * ahead, lambda c, _: start_a(c >> 4, c & 15), None)
        acc[...] = jnp.zeros_like(acc)
        if do_dma:
            pltpu.make_async_copy(x_buf, x_buf, w_sem.at[0]).wait()
            pltpu.make_async_copy(wq_buf, wq_buf, w_sem.at[1]).wait()
            pltpu.make_async_copy(wo_buf, wo_buf, w_sem.at[2]).wait()

        stream = [("b", c) for c in range(apos)] + [("a", c) for c in range(4)] + [("b", c) for c in range(apos, CPR)]
        n1 = sum(sched1)

        def start(m, kind, c):
            if kind == "a":
                u = m + REP + ahead
                pl.when(u < HQ)(lambda: start_a(u >> 2, (u & 3) * 4 + c))
            else:
                start_b(m, c)

        def q0_body(j, _):
            if do_dma:
                rest = stream[n1:]
                for i, (kind, c) in enumerate(rest):
                    @pl.when(j == i * REP // len(rest))
                    def _():
                        if kind == "a":
                            start_a(1, 4 * ahead + c)
                        else:
                            start_b(0, c)
            if do_compute:
                qa_buf[0, j] = project_q(0, j)
        lax.fori_loop(0, REP, q0_body, None)

        def part1(m):
            g, quarter = m >> 2, m & 3
            todo = stream[:n1]
            points = iter(sched1)

            def issue():
                mine = [todo.pop(0) for _ in range(next(points))]
                if not do_dma:
                    return
                for kind, c in mine:
                    start(m, kind, c)

            issue()
            if do_compute:
                qb_buf[m & 1] = project_q(1, m)
            issue()
            if do_compute:
                qa_buf[(g + 1) & 1, quarter] = project_q(0, jnp.minimum(m + REP, HQ - 1))

            if do_dma:
                @pl.when(quarter == 0)
                def _():
                    dst = kva_buf.at[g & 1]
                    pltpu.make_async_copy(dst, dst, a_sem.at[g & 1]).wait()

            oa = []
            for i in range(2):
                issue()
                if do_compute:
                    r0 = pl.multiple_of((2 * quarter + i) * (SQ // 2), SQ // 2)
                    q = qa_buf[g & 1, :, pl.ds(r0, SQ // 2)].reshape(REP * SQ // 2, DH)
                    s = scores(pltpu.bitcast(q, jnp.bfloat16), load(kva_buf.at[g & 1, quarter, 0, i]))
                issue()
                if do_compute:
                    o = weighted(softmax(s), load(kva_buf.at[g & 1, quarter, 1, i]))
                    oa.append(jnp.concatenate([o[j * SQ:(j + 1) * SQ] for j in range(REP)], axis=1))
            rows = pl.ds(pl.multiple_of(quarter * 2 * SQ, 2 * SQ), 2 * SQ)
            if do_compute:
                w = wo_buf[0, g >> 1, pl.ds(pl.multiple_of((g & 1) * GW, GW), GW)]
                acc[0, rows] += jnp.dot(jnp.concatenate(oa, axis=0).astype(jnp.bfloat16), w,
                                        preferred_element_type=jnp.float32)

            @pl.when(g == HKV - 1)
            def _():
                out_buf[0, rows] = acc[0, rows].astype(jnp.bfloat16)
                if not defer:
                    pltpu.make_async_copy(out_buf.at[0, rows], out_hbm.at[rows, pl.ds(0, D)], out_sem).start()

        def part2(h):
            slot = h & 1
            todo = stream[n1:]
            points = iter(sched2)

            def issue():
                mine = [todo.pop(0) for _ in range(next(points))]
                if do_dma and mine:
                    @pl.when(h + 1 < HQ)
                    def _():
                        for kind, c in mine:
                            start(h + 1, kind, c)

            def wait(p, a):
                if do_dma:
                    dst = kvb_buf.at[slot, p, a]
                    pltpu.make_async_copy(dst, dst, b_sem.at[(slot * NPAIR + p) * 2 + a]).wait()

            def qk(b):
                if b % 2 == 0:
                    wait(b // 2, 0)
                if do_compute:
                    q = pltpu.bitcast(qb_buf[slot, pl.ds(b * SQ // 2, SQ // 2)], jnp.bfloat16)
                    return scores(q, load(kvb_buf.at[slot, b // 2, 0, b % 2]))

            def send(t, r0, nr, prio):
                for j in range(osplit):
                    rows = pl.ds(r0 + j * nr // osplit, nr // osplit)
                    pltpu.make_async_copy(out_buf.at[t, rows], out_hbm.at[rows, pl.ds(t * D, D)], out_sem).start(priority=prio)

            def out_b(p):
                rows = pl.ds(p * 2 * SQ, 2 * SQ)
                if do_compute:
                    w = wo_buf[1, h >> 3, pl.ds(pl.multiple_of((h & 7) * DH, DH), DH)]
                    o = jnp.concatenate(ob[2 * p:2 * p + 2], axis=0).astype(jnp.bfloat16)
                    r = acc[1, rows] + jnp.dot(o, w, preferred_element_type=jnp.float32)
                    acc[1, rows] = r

                @pl.when(h == HQ - 1)
                def _():
                    if do_compute:
                        out_buf[1, rows] = r.astype(jnp.bfloat16)
                    if not defer or p == NPAIR - 1:
                        send(1, p * 2 * SQ, 2 * SQ, oprio[2])
                    elif p == NPAIR - 2:
                        if send1 == "o2":
                            send(0, 0, M, oprio[0])
                            send(1, 0, 6 * SQ, oprio[1])
                        else:
                            send(1, 4 * SQ, 2 * SQ, oprio[1])

            def send_early():
                @pl.when(h == HQ - 1)
                def _():
                    send(0, 0, M, oprio[0])
                    send(1, 0, 4 * SQ, oprio[1])

            def pv(b, pr):
                if do_compute:
                    ob.append(weighted(pr, load(kvb_buf.at[slot, b // 2, 1, b % 2])))

            def sm(b):
                if do_compute:
                    return softmax(sb[b])

            sb = [qk(0)]
            ob = []
            for b in range(B - 2):
                issue()
                sb.append(qk(b + 1))
                pr = sm(b)
                if b == 4 and early23:
                    out_b(1)
                    if send1 == "o1":
                        send_early()
                if b % 2 == 0:
                    wait(b // 2, 1)
                if b == 4 and send1 == "v2":
                    send_early()
                if b == 5 and send1 == "k3":
                    send_early()
                pv(b, pr)
                if b == 2:
                    out_b(0)
                if b == 4 and not early23:
                    out_b(1)
            issue()
            sb.append(qk(7))
            pr6 = sm(6)
            out_b(2)
            issue()
            pr7 = sm(7)
            wait(3, 1)
            pv(6, pr6)
            pv(7, pr7)
            out_b(3)

        def body(m, _):
            pl.when(m < HQ)(lambda: part1(m))
            pl.when(m > 0)(lambda: part2(m - 1))

        lax.fori_loop(0, HQ + 1, body, None)
        pltpu.make_async_copy(out_buf, out_buf, out_sem).wait()

    def f(A_x, A_k_cache, A_v_cache, A_wq, A_wo, B_x, B_k_cache, B_v_cache, B_wq, B_wo):
        out = pl.pallas_call(
            kernel, name=name,
            in_specs=[pl.BlockSpec(memory_space=pl.ANY)] * 10,
            out_specs=pl.BlockSpec(memory_space=pl.ANY),
            out_shape=jax.ShapeDtypeStruct((M, 2 * D), jnp.bfloat16),
            scratch_shapes=[
                pltpu.VMEM((2, M, D), jnp.bfloat16),
                pltpu.VMEM((2, 4, D // 4, HQ * DH), jnp.bfloat16),
                pltpu.VMEM((2, 4, HQ * DH // 4, D), jnp.bfloat16),
                pltpu.VMEM((2, NPAIR, 2, 2, SK, DH), jnp.bfloat16),
                pltpu.VMEM((2, NPAIR, 2, 2, SK, DH), jnp.bfloat16),
                pltpu.VMEM((2, REP, M // 2, DH), jnp.uint32),
                pltpu.VMEM((2, M // 2, DH), jnp.uint32),
                pltpu.VMEM((2, M, D), jnp.float32),
                pltpu.VMEM((2, M, D), jnp.bfloat16),
                pltpu.SemaphoreType.DMA((3,)),
                pltpu.SemaphoreType.DMA((2,)),
                pltpu.SemaphoreType.DMA((4 * NPAIR,)),
                pltpu.SemaphoreType.DMA(()),
            ],
            compiler_params=pltpu.CompilerParams(
                vmem_limit_bytes=vmem_mb * 2**20, disable_bounds_checks=not bchk,
                disable_semaphore_checks=not semchk, flags=flags),
        )(A_x.reshape(M, D), A_k_cache, A_v_cache, A_wq.reshape(4, D // 4, HQ * DH), A_wo.reshape(4, HQ * DH // 4, D),
          B_x.reshape(M, D), B_k_cache, B_v_cache, B_wq.reshape(4, D // 4, HQ * DH), B_wo.reshape(4, HQ * DH // 4, D))
        return out.reshape(B, SQ, 2 * D)
    return f


@jax.jit
def pallas_concat_heads__gqa_block_cached__mha_block_cached__near_ridge_kernel(
    A_x, A_k_cache, A_v_cache, A_wq, A_wo, B_x, B_k_cache, B_v_cache, B_wq, B_wo,
):
    return _build()(A_x, A_k_cache, A_v_cache, A_wq, A_wo, B_x, B_k_cache, B_v_cache, B_wq, B_wo)
```

```python
import jax
import jax.numpy as jnp
import numpy as np
from jax import lax
from jax.experimental import pallas as pl
from jax.experimental.pallas import tpu as pltpu

B, SQ, D = 8, 48, 512
HQ, HKV, SK, DH = 32, 8, 1024, 128
REP = HQ // HKV
M = B * SQ
NPAIR = B // 2
NCHUNK = 16
PIECE = SK // NCHUNK
WPART = 4
LAST_SPLIT = 6
GQA, MHA = 0, 1
QSCALE = float(DH ** -0.5 * np.log2(np.e))

STREAM = ([(MHA, c) for c in range(12)]
          + [(GQA, 0), (GQA, 1), (MHA, 12), (MHA, 13), (GQA, 2), (GQA, 3), (MHA, 14), (MHA, 15)])


def _rows(index, size):
    if isinstance(index, int):
        return pl.ds(index * size, size)
    return pl.ds(pl.multiple_of(index * size, size), size)


def _scores(q, k):
    return lax.dot_general(q, k, (((1,), (1,)), ((), ())), preferred_element_type=jnp.float32)


def _softmax(s):
    p = jnp.exp2(s - jnp.max(s, axis=1, keepdims=True))
    return p.astype(jnp.bfloat16), 1.0 / jnp.sum(p, axis=1, keepdims=True)


def _weighted(softmax, v):
    p, inv_sum = softmax
    return jnp.dot(p, v, preferred_element_type=jnp.float32) * inv_sum


def _kernel(xa_hbm, ka_hbm, va_hbm, wqa_hbm, woa_hbm, xb_hbm, kb_hbm, vb_hbm, wqb_hbm, wob_hbm,
            out_hbm,
            x_buf, wq_buf, wo_buf, kva_buf, kvb_buf, qa_buf, qb_buf, acc, out_buf,
            w_sem, a_sem, b_sem, out_sem):

    def wait_filled(dst, sem):
        pltpu.make_async_copy(dst, dst, sem).wait()

    def start_gqa(g, c):
        slot = g & 1
        rows = _rows(c, PIECE)
        for pair in (0, 2, 1, 3):
            for kv, src in enumerate((ka_hbm, va_hbm)):
                pltpu.make_async_copy(src.at[_rows(pair, 2), g, rows],
                                      kva_buf.at[slot, pair, kv, :, rows],
                                      a_sem.at[slot]).start(priority=kv)

    def last_sem(pair, kv, piece):
        return 2 + 2 * pair + kv + int(pair == NPAIR - 1 and kv == 1 and piece >= LAST_SPLIT)

    def start_mha(h, c):
        slot = h & 1
        last = h == HQ - 1
        for j in range(NPAIR):
            last_pair, last_piece = c // 4, 4 * (c % 4) + j
            pair = j if last_pair == j else jnp.where(last, last_pair, j)
            rows = _rows(c if last_piece == c else jnp.where(last, last_piece, c), PIECE)
            for kv, src in enumerate((kb_hbm, vb_hbm)):
                sem = jnp.where(last, last_sem(last_pair, kv, last_piece), slot)
                pltpu.make_async_copy(src.at[_rows(pair, 2), h, rows],
                                      kvb_buf.at[slot, pair, kv, :, rows],
                                      b_sem.at[sem]).start(priority=kv)

    def start(m, items):
        for block, c in items:
            if block == MHA:
                start_mha(m, c)
            else:
                quarter = m + REP + 1

                @pl.when(quarter < HQ)
                def _():
                    start_gqa(quarter >> 2, (quarter & 3) * 4 + c)

    def project_q(block, h):
        w = wq_buf[block, :, :, _rows(h, DH)].reshape(D, DH)
        q = jnp.dot(x_buf[block], w, preferred_element_type=jnp.float32)
        return (q * QSCALE).astype(jnp.bfloat16)

    for r in range(M // 32):
        for block, src in enumerate((xa_hbm, xb_hbm)):
            pltpu.make_async_copy(src.at[_rows(r, 32)], x_buf.at[block, _rows(r, 32)],
                                  w_sem.at[0]).start(priority=block)

    def start_weights(i, _):
        q_rows, q_cols, o_rows = _rows(i >> 2, 8), _rows(i & 3, 1024), _rows(i, 16)
        for half in range(2):
            parts = _rows(half, 2)
            for block, src in enumerate((wqa_hbm, wqb_hbm)):
                pltpu.make_async_copy(src.at[parts, q_rows, q_cols],
                                      wq_buf.at[block, parts, q_rows, q_cols],
                                      w_sem.at[1]).start(priority=block)
        for half in range(2):
            parts = _rows(half, 2)
            for block, src in enumerate((woa_hbm, wob_hbm)):
                pltpu.make_async_copy(src.at[parts, o_rows], wo_buf.at[block, parts, o_rows],
                                      w_sem.at[2]).start(priority=block)

    lax.fori_loop(0, 64, start_weights, None)
    lax.fori_loop(0, NCHUNK + 4, lambda c, _: start_gqa(c >> 4, c & 15), None)
    acc[...] = jnp.zeros_like(acc)
    wait_filled(x_buf, w_sem.at[0])
    wait_filled(wq_buf, w_sem.at[1])
    wait_filled(wo_buf, w_sem.at[2])

    def first_queries(j, _):
        start_gqa(1, 4 + j)
        rows = _rows(12 + j, PIECE)
        for pair in range(NPAIR):
            for kv, src in enumerate((kb_hbm, vb_hbm)):
                pltpu.make_async_copy(src.at[_rows(pair, 2), 0, rows],
                                      kvb_buf.at[0, pair, kv, :, rows],
                                      b_sem.at[0]).start(priority=kv)
        qa_buf[0, j] = project_q(GQA, j)

    lax.fori_loop(0, REP, first_queries, None)

    def gqa_part(m):
        g, pair = m >> 2, m & 3
        slot = g & 1

        @pl.when(pair == 0)
        def _():
            wait_filled(kva_buf.at[slot], a_sem.at[slot])

        def scores(i):
            q = qa_buf[slot, :, _rows(2 * pair + i, SQ)].reshape(REP * SQ, DH)
            return _scores(q, kva_buf[slot, pair, 0, i])

        def attend(i, s):
            o = _weighted(_softmax(s), kva_buf[slot, pair, 1, i])
            return jnp.concatenate([o[j * SQ:(j + 1) * SQ] for j in range(REP)], axis=1)

        start(m, STREAM[0:2])
        s0 = scores(0)
        start(m, STREAM[2:4])
        qb_buf[m & 1] = project_q(MHA, m)
        start(m, STREAM[4:6])
        o0 = attend(0, s0)
        start(m, STREAM[6:8])
        s1 = scores(1)
        start(m, STREAM[8:10])
        qa_buf[1 - slot, pair] = project_q(GQA, jnp.minimum(m + REP, HQ - 1))
        start(m, STREAM[10:12])
        o1 = attend(1, s1)
        o = jnp.concatenate([o0, o1], axis=0).astype(jnp.bfloat16)
        w = wo_buf[GQA, g >> 1, _rows(g & 1, REP * DH)]
        acc[GQA, _rows(pair, 2 * SQ)] += jnp.dot(o, w, preferred_element_type=jnp.float32)

    def mha_scores(h, b):
        return _scores(qb_buf[h & 1, _rows(b, SQ)], kvb_buf[h & 1, b // 2, 0, b % 2])

    def mha_weighted(h, b, softmax):
        return _weighted(softmax, kvb_buf[h & 1, b // 2, 1, b % 2])

    def mha_projected(h, rows, outs):
        o = jnp.concatenate(outs, axis=0).astype(jnp.bfloat16)
        w = wo_buf[MHA, h >> 3, _rows(h & 7, DH)]
        return acc[MHA, rows] + jnp.dot(o, w, preferred_element_type=jnp.float32)

    def mha_part(h):
        wait_filled(kvb_buf.at[h & 1], b_sem.at[h & 1])
        s = [mha_scores(h, 0), mha_scores(h, 1)]
        o = []
        for b in range(B):
            start(h + 1, STREAM[12 + b:13 + b])
            if b + 2 < B:
                s.append(mha_scores(h, b + 2))
            o.append(mha_weighted(h, b, _softmax(s[b])))
            if b == 5:
                acc[MHA, _rows(0, 4 * SQ)] = mha_projected(h, _rows(0, 4 * SQ), o[0:4])
        acc[MHA, _rows(1, 4 * SQ)] = mha_projected(h, _rows(1, 4 * SQ), o[4:8])

    def step(m, _):
        gqa_part(m)
        pl.when(m > 0)(lambda: mha_part(m - 1))

    lax.fori_loop(0, HQ, step, None)

    h = HQ - 1
    left, right = _rows(GQA, D), _rows(MHA, D)

    def wait_last(pair, kv):
        wait_filled(kvb_buf.at[h & 1, pair, kv], b_sem.at[last_sem(pair, kv, 0)])

    def wait_last_v(first, count):
        rows = pl.ds(first * PIECE, count * PIECE)
        wait_filled(kvb_buf.at[h & 1, NPAIR - 1, 1, :, rows], b_sem.at[last_sem(NPAIR - 1, 1, first)])

    def finish(pair, outs):
        rows = _rows(pair, 2 * SQ)
        out_buf[rows, right] = mha_projected(h, rows, outs).astype(jnp.bfloat16)

    sends = [pltpu.make_async_copy(out_buf.at[rows, cols], out_hbm.at[rows, cols], out_sem.at[i])
             for i, (rows, cols) in enumerate(((_rows(0, M), left), (_rows(0, 4 * SQ), right),
                                               (_rows(2, 2 * SQ), right), (_rows(3, 2 * SQ), right)))]

    out_buf[:, left] = acc[GQA].astype(jnp.bfloat16)
    for pair in range(3):
        wait_last(pair, 0)
    wait_last(0, 1)
    s = [mha_scores(h, b) for b in range(3)]
    o0 = mha_weighted(h, 0, _softmax(s[0]))
    s.append(mha_scores(h, 3))
    o1 = mha_weighted(h, 1, _softmax(s[1]))
    s.append(mha_scores(h, 4))
    p2 = _softmax(s[2])
    s.append(mha_scores(h, 5))
    p3 = _softmax(s[3])
    finish(0, [o0, o1])
    p4, p5 = _softmax(s[4]), _softmax(s[5])

    wait_last(1, 1)
    wait_last(3, 0)
    o2, o3 = mha_weighted(h, 2, p2), mha_weighted(h, 3, p3)
    s6, s7 = mha_scores(h, 6), mha_scores(h, 7)
    finish(1, [o2, o3])
    p6, p7 = _softmax(s6), _softmax(s7)

    wait_last(2, 1)
    wait_last_v(0, LAST_SPLIT)
    sends[0].start(priority=0)
    sends[1].start(priority=1)
    finish(2, [mha_weighted(h, 4, p4), mha_weighted(h, 5, p5)])
    sends[2].start(priority=1)

    wait_last_v(LAST_SPLIT, NCHUNK - LAST_SPLIT)
    finish(3, [mha_weighted(h, 6, p6), mha_weighted(h, 7, p7)])
    sends[3].start(priority=0)
    for send in sends:
        send.wait()


@jax.jit
def pallas_concat_heads__gqa_block_cached__mha_block_cached__near_ridge_kernel(
    A_x: jax.Array,
    A_k_cache: jax.Array,
    A_v_cache: jax.Array,
    A_wq: jax.Array,
    A_wo: jax.Array,
    B_x: jax.Array,
    B_k_cache: jax.Array,
    B_v_cache: jax.Array,
    B_wq: jax.Array,
    B_wo: jax.Array,
):
    wq_shape = (WPART, D // WPART, HQ * DH)
    wo_shape = (WPART, HQ * DH // WPART, D)
    kv_shape = (2, NPAIR, 2, 2, SK, DH)
    out = pl.pallas_call(
        _kernel,
        name="gqa_mha_cached_blocks",
        in_specs=[pl.BlockSpec(memory_space=pl.ANY)] * 10,
        out_specs=pl.BlockSpec(memory_space=pl.ANY),
        out_shape=jax.ShapeDtypeStruct((M, 2 * D), jnp.bfloat16),
        scratch_shapes=[
            pltpu.VMEM((2, M, D), jnp.bfloat16),
            pltpu.VMEM((2,) + wq_shape, jnp.bfloat16),
            pltpu.VMEM((2,) + wo_shape, jnp.bfloat16),
            pltpu.VMEM(kv_shape, jnp.bfloat16),
            pltpu.VMEM(kv_shape, jnp.bfloat16),
            pltpu.VMEM((2, REP, M, DH), jnp.bfloat16),
            pltpu.VMEM((2, M, DH), jnp.bfloat16),
            pltpu.VMEM((2, M, D), jnp.float32),
            pltpu.VMEM((M, 2 * D), jnp.bfloat16),
            pltpu.SemaphoreType.DMA((3,)),
            pltpu.SemaphoreType.DMA((2,)),
            pltpu.SemaphoreType.DMA((2 + 2 * NPAIR + 1,)),
            pltpu.SemaphoreType.DMA((4,)),
        ],
        compiler_params=pltpu.CompilerParams(
            vmem_limit_bytes=64 * 2**20,
            disable_semaphore_checks=True,
        ),
    )(A_x.reshape(M, D), A_k_cache, A_v_cache, A_wq.reshape(wq_shape), A_wo.reshape(wo_shape),
      B_x.reshape(M, D), B_k_cache, B_v_cache, B_wq.reshape(wq_shape), B_wo.reshape(wo_shape))
    return out.reshape(B, SQ, 2 * D)
```

```python
import jax
import jax.numpy as jnp
import numpy as np
from jax import lax
from jax.experimental import pallas as pl
from jax.experimental.pallas import tpu as pltpu

B, SQ, D = 8, 48, 512
HQ, HKV, SK, DH = 32, 8, 1024, 128
REP = HQ // HKV
M = B * SQ
NPAIR = B // 2
NCHUNK = 16
PIECE = SK // NCHUNK
WPART = 4
LAST_SPLIT = 6
GQA, MHA = 0, 1
QSCALE = float(DH ** -0.5 * np.log2(np.e))

STARTS_IN_GQA_PART = [[(MHA, c) for c in cs]
                      for cs in ((0, 1), (2, 3), (4, 5), (6, 7), (8, 9), (10,), (11, 12, 13))]
STARTS_IN_MHA_PART = [[(GQA, 0)], [(GQA, 1)], [(GQA, 2)], [], [(GQA, 3)], [(MHA, 14)], [(MHA, 15)], []]


def _rows(index, size):
    if isinstance(index, int):
        return pl.ds(index * size, size)
    return pl.ds(pl.multiple_of(index * size, size), size)


def _scores(q, k):
    return lax.dot_general(q, k, (((1,), (1,)), ((), ())), preferred_element_type=jnp.float32)


def _softmax(s):
    p = jnp.exp2(s - jnp.max(s, axis=1, keepdims=True))
    return p.astype(jnp.bfloat16), 1.0 / jnp.sum(p, axis=1, keepdims=True)


def _weighted(softmax, v):
    p, inv_sum = softmax
    return jnp.dot(p, v, preferred_element_type=jnp.float32) * inv_sum


def _kernel(xa_hbm, ka_hbm, va_hbm, wqa_hbm, woa_hbm, xb_hbm, kb_hbm, vb_hbm, wqb_hbm, wob_hbm,
            out_hbm,
            x_buf, wq_buf, wo_buf, kv_buf, qa_buf, qb_buf, acc, out_buf,
            w_sem, a_sem, b_sem, out_sem):

    def wait_filled(dst, sem):
        pltpu.make_async_copy(dst, dst, sem).wait()

    def start_gqa(g, c):
        slot = g & 1
        rows = _rows(c, PIECE)
        for pair in (0, 2, 1, 3):
            for kv, src in enumerate((ka_hbm, va_hbm)):
                pltpu.make_async_copy(src.at[_rows(pair, 2), g, rows],
                                      kv_buf.at[2 + slot, pair, kv, :, rows],
                                      a_sem.at[slot]).start(priority=kv)

    def last_sem(pair, kv, piece):
        return 2 + 2 * pair + kv + int(pair == NPAIR - 1 and kv == 1 and piece >= LAST_SPLIT)

    def start_mha(h, c):
        slot = h & 1

        def pick(in_last_round, otherwise):
            if isinstance(h, int):
                return in_last_round if h == HQ - 1 else otherwise
            if isinstance(otherwise, int) and otherwise == in_last_round:
                return otherwise
            return jnp.where(h == HQ - 1, in_last_round, otherwise)

        for j in range(NPAIR):
            last_pair, last_piece = c // 4, 4 * (c % 4) + j
            pair = pick(last_pair, j)
            rows = _rows(pick(last_piece, c), PIECE)
            for kv, src in enumerate((kb_hbm, vb_hbm)):
                sem = pick(last_sem(last_pair, kv, last_piece), slot)
                pltpu.make_async_copy(src.at[_rows(pair, 2), h, rows],
                                      kv_buf.at[slot, pair, kv, :, rows],
                                      b_sem.at[sem]).start(priority=kv)

    def start(m, items):
        for block, c in items:
            if block == MHA:
                start_mha(m, c)
            else:
                quarter = m + REP + 1

                @pl.when(quarter < HQ)
                def _():
                    start_gqa(quarter >> 2, (quarter & 3) * 4 + c)

    def project_q(block, h):
        w = wq_buf[block, :, :, _rows(h, DH)].reshape(D, DH)
        q = jnp.dot(x_buf[block], w, preferred_element_type=jnp.float32)
        return (q * QSCALE).astype(jnp.bfloat16)

    for r in range(M // 32):
        for block, src in enumerate((xa_hbm, xb_hbm)):
            pltpu.make_async_copy(src.at[_rows(r, 32)], x_buf.at[block, _rows(r, 32)],
                                  w_sem.at[0]).start(priority=block)

    def start_weights(i, _):
        q_rows, q_cols, o_rows = _rows(i >> 2, 8), _rows(i & 3, 1024), _rows(i, 16)
        for half in range(2):
            parts = _rows(half, 2)
            for block, src in enumerate((wqa_hbm, wqb_hbm)):
                pltpu.make_async_copy(src.at[parts, q_rows, q_cols],
                                      wq_buf.at[block, parts, q_rows, q_cols],
                                      w_sem.at[1]).start(priority=block)
        for half in range(2):
            parts = _rows(half, 2)
            for block, src in enumerate((woa_hbm, wob_hbm)):
                pltpu.make_async_copy(src.at[parts, o_rows], wo_buf.at[block, parts, o_rows],
                                      w_sem.at[2]).start(priority=block)

    lax.fori_loop(0, 64, start_weights, None)
    acc[...] = jnp.zeros_like(acc)
    lax.fori_loop(0, NCHUNK + 4, lambda c, _: start_gqa(c >> 4, c & 15), None)
    wait_filled(x_buf, w_sem.at[0])
    wait_filled(wq_buf, w_sem.at[1])
    wait_filled(wo_buf, w_sem.at[2])

    def first_queries(j, _):
        @pl.when(j < 2)
        def _():
            start_gqa(1, 4 + 2 * j)
            start_gqa(1, 5 + 2 * j)

        @pl.when(j == 2)
        def _():
            start_mha(0, 14)
            start_mha(0, 15)

        qa_buf[0, j] = project_q(GQA, j)

    lax.fori_loop(0, REP, first_queries, None)

    def gqa_part(m):
        g, pair = m >> 2, m & 3
        slot = g & 1

        @pl.when(pair == 0)
        def _():
            wait_filled(kv_buf.at[2 + slot], a_sem.at[slot])

        def scores(i):
            q = qa_buf[slot, :, _rows(2 * pair + i, SQ)].reshape(REP * SQ, DH)
            return _scores(q, kv_buf[2 + slot, pair, 0, i])

        def attend(i, s):
            o = _weighted(_softmax(s), kv_buf[2 + slot, pair, 1, i])
            return jnp.concatenate([o[j * SQ:(j + 1) * SQ] for j in range(REP)], axis=1)

        start(m, STARTS_IN_GQA_PART[0])
        s0 = scores(0)
        start(m, STARTS_IN_GQA_PART[1])
        qb_buf[m & 1] = project_q(MHA, m)
        start(m, STARTS_IN_GQA_PART[2])
        o0 = attend(0, s0)
        start(m, STARTS_IN_GQA_PART[3])
        s1 = scores(1)
        start(m, STARTS_IN_GQA_PART[4])
        qa_buf[1 - slot, pair] = project_q(GQA, jnp.minimum(m + REP, HQ - 1))
        start(m, STARTS_IN_GQA_PART[5])
        o1 = attend(1, s1)
        start(m, STARTS_IN_GQA_PART[6])
        o = jnp.concatenate([o0, o1], axis=0).astype(jnp.bfloat16)
        w = wo_buf[GQA, g >> 1, _rows(g & 1, REP * DH)]
        acc[GQA, _rows(pair, 2 * SQ)] += jnp.dot(o, w, preferred_element_type=jnp.float32)

    def mha_scores(h, b):
        return _scores(qb_buf[h & 1, _rows(b, SQ)], kv_buf[h & 1, b // 2, 0, b % 2])

    def mha_weighted(h, b, softmax):
        return _weighted(softmax, kv_buf[h & 1, b // 2, 1, b % 2])

    def mha_projected(h, rows, outs):
        o = jnp.concatenate(outs, axis=0).astype(jnp.bfloat16)
        w = wo_buf[MHA, h >> 3, _rows(h & 7, DH)]
        return acc[MHA, rows] + jnp.dot(o, w, preferred_element_type=jnp.float32)

    def mha_part(h):
        wait_filled(kv_buf.at[h & 1], b_sem.at[h & 1])
        s = [mha_scores(h, 0), mha_scores(h, 1)]
        o = []
        for b in range(B):
            start(h + 1, STARTS_IN_MHA_PART[b])
            if b + 2 < B:
                s.append(mha_scores(h, b + 2))
            o.append(mha_weighted(h, b, _softmax(s[b])))
            if b == 5:
                acc[MHA, _rows(0, 4 * SQ)] = mha_projected(h, _rows(0, 4 * SQ), o[0:4])
        acc[MHA, _rows(1, 4 * SQ)] = mha_projected(h, _rows(1, 4 * SQ), o[4:8])

    def step(m, _):
        gqa_part(m)
        pl.when(m > 0)(lambda: mha_part(m - 1))

    lax.fori_loop(0, HQ, step, None)

    h = HQ - 1
    left, right = _rows(GQA, D), _rows(MHA, D)

    def wait_last(pair, kv):
        wait_filled(kv_buf.at[h & 1, pair, kv], b_sem.at[last_sem(pair, kv, 0)])

    def wait_last_v(first, count):
        rows = pl.ds(first * PIECE, count * PIECE)
        wait_filled(kv_buf.at[h & 1, NPAIR - 1, 1, :, rows], b_sem.at[last_sem(NPAIR - 1, 1, first)])

    def finish(pair, outs):
        rows = _rows(pair, 2 * SQ)
        out_buf[rows, right] = mha_projected(h, rows, outs).astype(jnp.bfloat16)

    sends = [pltpu.make_async_copy(out_buf.at[rows, cols], out_hbm.at[rows, cols], out_sem.at[i])
             for i, (rows, cols) in enumerate(((_rows(0, M), left), (_rows(0, 4 * SQ), right),
                                               (_rows(2, 2 * SQ), right), (_rows(3, 2 * SQ), right)))]

    out_buf[:, left] = acc[GQA].astype(jnp.bfloat16)
    for pair in range(3):
        wait_last(pair, 0)
    wait_last(0, 1)
    s = [mha_scores(h, b) for b in range(3)]
    o0 = mha_weighted(h, 0, _softmax(s[0]))
    s.append(mha_scores(h, 3))
    o1 = mha_weighted(h, 1, _softmax(s[1]))
    s.append(mha_scores(h, 4))
    p2 = _softmax(s[2])
    s.append(mha_scores(h, 5))
    p3 = _softmax(s[3])
    finish(0, [o0, o1])
    p4, p5 = _softmax(s[4]), _softmax(s[5])

    wait_last(1, 1)
    wait_last(3, 0)
    o2, o3 = mha_weighted(h, 2, p2), mha_weighted(h, 3, p3)
    s6, s7 = mha_scores(h, 6), mha_scores(h, 7)
    finish(1, [o2, o3])
    p6, p7 = _softmax(s6), _softmax(s7)

    wait_last(2, 1)
    wait_last_v(0, LAST_SPLIT)
    sends[0].start(priority=0)
    sends[1].start(priority=1)
    finish(2, [mha_weighted(h, 4, p4), mha_weighted(h, 5, p5)])
    sends[2].start(priority=1)

    wait_last_v(LAST_SPLIT, NCHUNK - LAST_SPLIT)
    finish(3, [mha_weighted(h, 6, p6), mha_weighted(h, 7, p7)])
    sends[3].start(priority=0)
    for send in sends:
        send.wait()


@jax.jit
def pallas_concat_heads__gqa_block_cached__mha_block_cached__near_ridge_kernel(
    A_x: jax.Array,
    A_k_cache: jax.Array,
    A_v_cache: jax.Array,
    A_wq: jax.Array,
    A_wo: jax.Array,
    B_x: jax.Array,
    B_k_cache: jax.Array,
    B_v_cache: jax.Array,
    B_wq: jax.Array,
    B_wo: jax.Array,
):
    wq_shape = (WPART, D // WPART, HQ * DH)
    wo_shape = (WPART, HQ * DH // WPART, D)
    kv_shape = (4, NPAIR, 2, 2, SK, DH)
    out = pl.pallas_call(
        _kernel,
        name="gqa_mha_cached_blocks",
        in_specs=[pl.BlockSpec(memory_space=pl.ANY)] * 10,
        out_specs=pl.BlockSpec(memory_space=pl.ANY),
        out_shape=jax.ShapeDtypeStruct((M, 2 * D), jnp.bfloat16),
        scratch_shapes=[
            pltpu.VMEM((2, M, D), jnp.bfloat16),
            pltpu.VMEM((2,) + wq_shape, jnp.bfloat16),
            pltpu.VMEM((2,) + wo_shape, jnp.bfloat16),
            pltpu.VMEM(kv_shape, jnp.bfloat16),
            pltpu.VMEM((2, REP, M, DH), jnp.bfloat16),
            pltpu.VMEM((2, M, DH), jnp.bfloat16),
            pltpu.VMEM((2, M, D), jnp.float32),
            pltpu.VMEM((M, 2 * D), jnp.bfloat16),
            pltpu.SemaphoreType.DMA((3,)),
            pltpu.SemaphoreType.DMA((2,)),
            pltpu.SemaphoreType.DMA((2 + 2 * NPAIR + 1,)),
            pltpu.SemaphoreType.DMA((4,)),
        ],
        compiler_params=pltpu.CompilerParams(
            vmem_limit_bytes=64 * 2**20,
            disable_semaphore_checks=True,
        ),
    )(A_x.reshape(M, D), A_k_cache, A_v_cache, A_wq.reshape(wq_shape), A_wo.reshape(wo_shape),
      B_x.reshape(M, D), B_k_cache, B_v_cache, B_wq.reshape(wq_shape), B_wo.reshape(wo_shape))
    return out.reshape(B, SQ, 2 * D)
```

```python
import jax
import jax.numpy as jnp
import numpy as np
from jax import lax
from jax.experimental import pallas as pl
from jax.experimental.pallas import tpu as pltpu

B, SQ, D = 8, 48, 512
HQ, HKV, SK, DH = 32, 8, 1024, 128
REP = HQ // HKV
M = B * SQ
NPAIR = B // 2
NCHUNK = 16
PIECE = SK // NCHUNK
WPART = 4
LAST_SPLIT = 6
GQA, MHA = 0, 1
SCALE = float(DH ** -0.5 * np.log2(np.e))

STARTS_IN_GQA_PART = [[(MHA, c) for c in cs]
                      for cs in ((0, 1), (2, 3), (4, 5), (6, 7), (8, 9), (10,), (11, 12, 13))]
STARTS_IN_MHA_PART = [[(GQA, 0)], [(GQA, 1)], [(GQA, 2)], [], [(GQA, 3)], [(MHA, 14)], [(MHA, 15)], []]


def _rows(index, size):
    if isinstance(index, int):
        return pl.ds(index * size, size)
    return pl.ds(pl.multiple_of(index * size, size), size)


def _scores(q, k):
    return lax.dot_general(q, k, (((1,), (1,)), ((), ())), preferred_element_type=jnp.float32)


def _softmax(s):
    p = jnp.exp2((s - jnp.max(s, axis=1, keepdims=True)) * SCALE)
    return p.astype(jnp.bfloat16), 1.0 / jnp.sum(p, axis=1, keepdims=True)


def _weighted(softmax, v):
    p, inv_sum = softmax
    return jnp.dot(p, v, preferred_element_type=jnp.float32) * inv_sum


def _kernel(xa_hbm, ka_hbm, va_hbm, wqa_hbm, woa_hbm, xb_hbm, kb_hbm, vb_hbm, wqb_hbm, wob_hbm,
            out_hbm,
            x_buf, wq_buf, wo_buf, kv_buf, qa_buf, qb_buf, acc, out_buf,
            w_sem, a_sem, b_sem, out_sem):

    def wait_filled(dst, sem):
        pltpu.make_async_copy(dst, dst, sem).wait()

    def start_gqa(g, c):
        slot = g & 1
        rows = _rows(c, PIECE)
        for pair in (0, 2, 1, 3):
            for kv, src in enumerate((ka_hbm, va_hbm)):
                pltpu.make_async_copy(src.at[_rows(pair, 2), g, rows],
                                      kv_buf.at[2 + slot, pair, kv, :, rows],
                                      a_sem.at[slot]).start(priority=kv)

    def last_sem(pair, kv, piece):
        return 2 + 2 * pair + kv + int(pair == NPAIR - 1 and kv == 1 and piece >= LAST_SPLIT)

    def start_mha(h, c):
        slot = h & 1

        def pick(in_last_round, otherwise):
            if isinstance(h, int):
                return in_last_round if h == HQ - 1 else otherwise
            if isinstance(otherwise, int) and otherwise == in_last_round:
                return otherwise
            return jnp.where(h == HQ - 1, in_last_round, otherwise)

        for j in range(NPAIR):
            last_pair, last_piece = c // 4, 4 * (c % 4) + j
            pair = pick(last_pair, j)
            rows = _rows(pick(last_piece, c), PIECE)
            for kv, src in enumerate((kb_hbm, vb_hbm)):
                sem = pick(last_sem(last_pair, kv, last_piece), slot)
                pltpu.make_async_copy(src.at[_rows(pair, 2), h, rows],
                                      kv_buf.at[slot, pair, kv, :, rows],
                                      b_sem.at[sem]).start(priority=kv)

    def start(m, items):
        for block, c in items:
            if block == MHA:
                start_mha(m, c)
            else:
                quarter = m + REP + 1

                @pl.when(quarter < HQ)
                def _():
                    start_gqa(quarter >> 2, (quarter & 3) * 4 + c)

    def project_q(block, h):
        w = wq_buf[block, :, :, _rows(h, DH)].reshape(D, DH)
        return jnp.dot(x_buf[block], w, preferred_element_type=jnp.float32).astype(jnp.bfloat16)

    for r in range(M // 32):
        for block, src in enumerate((xa_hbm, xb_hbm)):
            pltpu.make_async_copy(src.at[_rows(r, 32)], x_buf.at[block, _rows(r, 32)],
                                  w_sem.at[0]).start(priority=block)

    def start_weights(i, _):
        q_rows, q_cols, o_rows = _rows(i >> 2, 8), _rows(i & 3, 1024), _rows(i, 16)
        for half in range(2):
            parts = _rows(half, 2)
            for block, src in enumerate((wqa_hbm, wqb_hbm)):
                pltpu.make_async_copy(src.at[parts, q_rows, q_cols],
                                      wq_buf.at[block, parts, q_rows, q_cols],
                                      w_sem.at[1]).start(priority=block)
        for half in range(2):
            parts = _rows(half, 2)
            for block, src in enumerate((woa_hbm, wob_hbm)):
                pltpu.make_async_copy(src.at[parts, o_rows], wo_buf.at[block, parts, o_rows],
                                      w_sem.at[2]).start(priority=block)

    lax.fori_loop(0, 64, start_weights, None)
    acc[...] = jnp.zeros_like(acc)
    lax.fori_loop(0, NCHUNK + 4, lambda c, _: start_gqa(c >> 4, c & 15), None)
    wait_filled(x_buf, w_sem.at[0])
    wait_filled(wq_buf, w_sem.at[1])
    wait_filled(wo_buf, w_sem.at[2])

    def first_queries(j, _):
        @pl.when(j < 2)
        def _():
            start_gqa(1, 4 + 2 * j)
            start_gqa(1, 5 + 2 * j)

        @pl.when(j == 2)
        def _():
            start_mha(0, 14)
            start_mha(0, 15)

        qa_buf[0, j] = project_q(GQA, j)

    lax.fori_loop(0, REP, first_queries, None)

    def gqa_part(m):
        g, pair = m >> 2, m & 3
        slot = g & 1

        @pl.when(pair == 0)
        def _():
            wait_filled(kv_buf.at[2 + slot], a_sem.at[slot])

        def scores(i):
            q = qa_buf[slot, :, _rows(2 * pair + i, SQ)].reshape(REP * SQ, DH)
            return _scores(q, kv_buf[2 + slot, pair, 0, i])

        def attend(i, s):
            o = _weighted(_softmax(s), kv_buf[2 + slot, pair, 1, i])
            return jnp.concatenate([o[j * SQ:(j + 1) * SQ] for j in range(REP)], axis=1)

        start(m, STARTS_IN_GQA_PART[0])
        s0 = scores(0)
        start(m, STARTS_IN_GQA_PART[1])
        qb_buf[m & 1] = project_q(MHA, m)
        start(m, STARTS_IN_GQA_PART[2])
        o0 = attend(0, s0)
        start(m, STARTS_IN_GQA_PART[3])
        s1 = scores(1)
        start(m, STARTS_IN_GQA_PART[4])
        qa_buf[1 - slot, pair] = project_q(GQA, jnp.minimum(m + REP, HQ - 1))
        start(m, STARTS_IN_GQA_PART[5])
        o1 = attend(1, s1)
        start(m, STARTS_IN_GQA_PART[6])
        o = jnp.concatenate([o0, o1], axis=0).astype(jnp.bfloat16)
        w = wo_buf[GQA, g >> 1, _rows(g & 1, REP * DH)]
        acc[GQA, _rows(pair, 2 * SQ)] += jnp.dot(o, w, preferred_element_type=jnp.float32)

    def mha_scores(h, b):
        return _scores(qb_buf[h & 1, _rows(b, SQ)], kv_buf[h & 1, b // 2, 0, b % 2])

    def mha_weighted(h, b, softmax):
        return _weighted(softmax, kv_buf[h & 1, b // 2, 1, b % 2])

    def mha_projected(h, rows, outs):
        o = jnp.concatenate(outs, axis=0).astype(jnp.bfloat16)
        w = wo_buf[MHA, h >> 3, _rows(h & 7, DH)]
        return acc[MHA, rows] + jnp.dot(o, w, preferred_element_type=jnp.float32)

    def mha_part(h):
        wait_filled(kv_buf.at[h & 1], b_sem.at[h & 1])
        s = [mha_scores(h, 0), mha_scores(h, 1)]
        o = []
        for b in range(B):
            start(h + 1, STARTS_IN_MHA_PART[b])
            if b + 2 < B:
                s.append(mha_scores(h, b + 2))
            o.append(mha_weighted(h, b, _softmax(s[b])))
            if b == 5:
                acc[MHA, _rows(0, 4 * SQ)] = mha_projected(h, _rows(0, 4 * SQ), o[0:4])
        acc[MHA, _rows(1, 4 * SQ)] = mha_projected(h, _rows(1, 4 * SQ), o[4:8])

    def step(m, _):
        gqa_part(m)
        pl.when(m > 0)(lambda: mha_part(m - 1))

    lax.fori_loop(0, HQ, step, None)

    h = HQ - 1
    left, right = _rows(GQA, D), _rows(MHA, D)

    def wait_last(pair, kv):
        wait_filled(kv_buf.at[h & 1, pair, kv], b_sem.at[last_sem(pair, kv, 0)])

    def wait_last_v(first, count):
        rows = pl.ds(first * PIECE, count * PIECE)
        wait_filled(kv_buf.at[h & 1, NPAIR - 1, 1, :, rows], b_sem.at[last_sem(NPAIR - 1, 1, first)])

    def finish(pair, outs):
        rows = _rows(pair, 2 * SQ)
        out_buf[rows, right] = mha_projected(h, rows, outs).astype(jnp.bfloat16)

    sends = [pltpu.make_async_copy(out_buf.at[rows, cols], out_hbm.at[rows, cols], out_sem.at[i])
             for i, (rows, cols) in enumerate(((_rows(0, M), left), (_rows(0, 4 * SQ), right),
                                               (_rows(2, 2 * SQ), right), (_rows(3, 2 * SQ), right)))]

    out_buf[:, left] = acc[GQA].astype(jnp.bfloat16)
    for pair in range(3):
        wait_last(pair, 0)
    wait_last(0, 1)
    s = [mha_scores(h, b) for b in range(3)]
    o0 = mha_weighted(h, 0, _softmax(s[0]))
    s.append(mha_scores(h, 3))
    o1 = mha_weighted(h, 1, _softmax(s[1]))
    s.append(mha_scores(h, 4))
    p2 = _softmax(s[2])
    s.append(mha_scores(h, 5))
    p3 = _softmax(s[3])
    finish(0, [o0, o1])
    p4, p5 = _softmax(s[4]), _softmax(s[5])

    wait_last(1, 1)
    wait_last(3, 0)
    o2, o3 = mha_weighted(h, 2, p2), mha_weighted(h, 3, p3)
    s6, s7 = mha_scores(h, 6), mha_scores(h, 7)
    finish(1, [o2, o3])
    p6, p7 = _softmax(s6), _softmax(s7)

    wait_last(2, 1)
    wait_last_v(0, LAST_SPLIT)
    sends[0].start(priority=0)
    sends[1].start(priority=1)
    finish(2, [mha_weighted(h, 4, p4), mha_weighted(h, 5, p5)])
    sends[2].start(priority=1)

    wait_last_v(LAST_SPLIT, NCHUNK - LAST_SPLIT)
    finish(3, [mha_weighted(h, 6, p6), mha_weighted(h, 7, p7)])
    sends[3].start(priority=0)
    for send in sends:
        send.wait()


@jax.jit
def pallas_concat_heads__gqa_block_cached__mha_block_cached__near_ridge_kernel(
    A_x: jax.Array,
    A_k_cache: jax.Array,
    A_v_cache: jax.Array,
    A_wq: jax.Array,
    A_wo: jax.Array,
    B_x: jax.Array,
    B_k_cache: jax.Array,
    B_v_cache: jax.Array,
    B_wq: jax.Array,
    B_wo: jax.Array,
):
    wq_shape = (WPART, D // WPART, HQ * DH)
    wo_shape = (WPART, HQ * DH // WPART, D)
    kv_shape = (4, NPAIR, 2, 2, SK, DH)
    out = pl.pallas_call(
        _kernel,
        name="gqa_mha_cached_blocks",
        in_specs=[pl.BlockSpec(memory_space=pl.ANY)] * 10,
        out_specs=pl.BlockSpec(memory_space=pl.ANY),
        out_shape=jax.ShapeDtypeStruct((M, 2 * D), jnp.bfloat16),
        scratch_shapes=[
            pltpu.VMEM((2, M, D), jnp.bfloat16),
            pltpu.VMEM((2,) + wq_shape, jnp.bfloat16),
            pltpu.VMEM((2,) + wo_shape, jnp.bfloat16),
            pltpu.VMEM(kv_shape, jnp.bfloat16),
            pltpu.VMEM((2, REP, M, DH), jnp.bfloat16),
            pltpu.VMEM((2, M, DH), jnp.bfloat16),
            pltpu.VMEM((2, M, D), jnp.float32),
            pltpu.VMEM((M, 2 * D), jnp.bfloat16),
            pltpu.SemaphoreType.DMA((3,)),
            pltpu.SemaphoreType.DMA((2,)),
            pltpu.SemaphoreType.DMA((2 + 2 * NPAIR + 1,)),
            pltpu.SemaphoreType.DMA((4,)),
        ],
        compiler_params=pltpu.CompilerParams(
            vmem_limit_bytes=64 * 2**20,
            disable_semaphore_checks=True,
        ),
    )(A_x.reshape(M, D), A_k_cache, A_v_cache, A_wq.reshape(wq_shape), A_wo.reshape(wo_shape),
      B_x.reshape(M, D), B_k_cache, B_v_cache, B_wq.reshape(wq_shape), B_wo.reshape(wo_shape))
    return out.reshape(B, SQ, 2 * D)
```

```python
import functools

import jax
import jax.numpy as jnp
import numpy as np
from jax import lax
from jax.experimental import pallas as pl
from jax.experimental.pallas import tpu as pltpu

B, SQ, D = 8, 48, 512
HQ, HKV, SK, DH = 32, 8, 1024, 128
REP = HQ // HKV
M = B * SQ
NPAIR = B // 2
NCHUNK = 16
PIECE = SK // NCHUNK
WPART = 4
LAST_SPLIT = 6
GQA, MHA = 0, 1
SCALE = float(DH ** -0.5 * np.log2(np.e))

STARTS_IN_GQA_PART = [[(MHA, c) for c in cs]
                      for cs in ((0, 1), (2, 3), (4, 5), (6, 7), (8, 9), (10,), (11, 12, 13))]
STARTS_IN_MHA_PART = [[(GQA, 0)], [(GQA, 1)], [(GQA, 2)], [], [(GQA, 3)], [(MHA, 14)], [(MHA, 15)], []]


def _rows(index, size):
    if isinstance(index, int):
        return pl.ds(index * size, size)
    return pl.ds(pl.multiple_of(index * size, size), size)


def _scores(q, k):
    return lax.dot_general(q, k, (((1,), (1,)), ((), ())), preferred_element_type=jnp.float32)


def _softmax(s):
    p = jnp.exp2((s - jnp.max(s, axis=1, keepdims=True)) * SCALE)
    return p.astype(jnp.bfloat16), 1.0 / jnp.sum(p, axis=1, keepdims=True)


def _weighted(softmax, v):
    p, inv_sum = softmax
    return jnp.dot(p, v, preferred_element_type=jnp.float32) * inv_sum


def _output_copies(out_buf, out_hbm, out_sem):
    left, right = _rows(GQA, D), _rows(MHA, D)
    return [pltpu.make_async_copy(out_buf.at[rows, cols], out_hbm.at[rows, cols], out_sem)
            for rows, cols in ((_rows(0, M), left), (_rows(0, 4 * SQ), right),
                               (_rows(2, 2 * SQ), right), (_rows(3, 2 * SQ), right))]


def _kernel(*refs):
    out_hbm, out_buf, out_sem = refs[10], refs[-2], refs[-1]
    pl.run_scoped(functools.partial(_compute, *refs),
                  pltpu.SemaphoreType.DMA((3,)),
                  pltpu.SemaphoreType.DMA((2,)),
                  pltpu.SemaphoreType.DMA((2 + 2 * NPAIR + 1,)))
    for copy in _output_copies(out_buf, out_hbm, out_sem):
        copy.wait()


def _compute(xa_hbm, ka_hbm, va_hbm, wqa_hbm, woa_hbm, xb_hbm, kb_hbm, vb_hbm, wqb_hbm, wob_hbm,
             out_hbm,
             x_buf, wq_buf, wo_buf, kv_buf, qa_buf, qb_buf, acc, out_buf, out_sem,
             w_sem, a_sem, b_sem):

    def wait_filled(dst, sem):
        pltpu.make_async_copy(dst, dst, sem).wait()

    def start_gqa(g, c):
        slot = g & 1
        rows = _rows(c, PIECE)
        for pair in (0, 2, 1, 3):
            for kv, src in enumerate((ka_hbm, va_hbm)):
                pltpu.make_async_copy(src.at[_rows(pair, 2), g, rows],
                                      kv_buf.at[2 + slot, pair, kv, :, rows],
                                      a_sem.at[slot]).start(priority=kv)

    def last_sem(pair, kv, piece):
        return 2 + 2 * pair + kv + int(pair == NPAIR - 1 and kv == 1 and piece >= LAST_SPLIT)

    def start_mha(h, c):
        slot = h & 1

        def pick(in_last_round, otherwise):
            if isinstance(h, int):
                return in_last_round if h == HQ - 1 else otherwise
            if isinstance(otherwise, int) and otherwise == in_last_round:
                return otherwise
            return jnp.where(h == HQ - 1, in_last_round, otherwise)

        for j in range(NPAIR):
            last_pair, last_piece = c // 4, 4 * (c % 4) + j
            pair = pick(last_pair, j)
            rows = _rows(pick(last_piece, c), PIECE)
            for kv, src in enumerate((kb_hbm, vb_hbm)):
                sem = pick(last_sem(last_pair, kv, last_piece), slot)
                pltpu.make_async_copy(src.at[_rows(pair, 2), h, rows],
                                      kv_buf.at[slot, pair, kv, :, rows],
                                      b_sem.at[sem]).start(priority=kv)

    def start(m, items):
        for block, c in items:
            if block == MHA:
                start_mha(m, c)
            else:
                quarter = m + REP + 1

                @pl.when(quarter < HQ)
                def _():
                    start_gqa(quarter >> 2, (quarter & 3) * 4 + c)

    def project_q(block, h):
        w = wq_buf[block, :, :, _rows(h, DH)].reshape(D, DH)
        return jnp.dot(x_buf[block], w, preferred_element_type=jnp.float32).astype(jnp.bfloat16)

    for r in range(M // 32):
        for block, src in enumerate((xa_hbm, xb_hbm)):
            pltpu.make_async_copy(src.at[_rows(r, 32)], x_buf.at[block, _rows(r, 32)],
                                  w_sem.at[0]).start(priority=block)

    def start_weights(i, _):
        q_rows, q_cols, o_rows = _rows(i >> 2, 8), _rows(i & 3, 1024), _rows(i, 16)
        for half in range(2):
            parts = _rows(half, 2)
            for block, src in enumerate((wqa_hbm, wqb_hbm)):
                pltpu.make_async_copy(src.at[parts, q_rows, q_cols],
                                      wq_buf.at[block, parts, q_rows, q_cols],
                                      w_sem.at[1]).start(priority=block)
        for half in range(2):
            parts = _rows(half, 2)
            for block, src in enumerate((woa_hbm, wob_hbm)):
                pltpu.make_async_copy(src.at[parts, o_rows], wo_buf.at[block, parts, o_rows],
                                      w_sem.at[2]).start(priority=block)

    lax.fori_loop(0, 64, start_weights, None)
    acc[...] = jnp.zeros_like(acc)
    lax.fori_loop(0, NCHUNK + 4, lambda c, _: start_gqa(c >> 4, c & 15), None)
    wait_filled(x_buf, w_sem.at[0])
    wait_filled(wq_buf, w_sem.at[1])
    wait_filled(wo_buf, w_sem.at[2])

    def first_queries(j, _):
        @pl.when(j < 2)
        def _():
            start_gqa(1, 4 + 2 * j)
            start_gqa(1, 5 + 2 * j)

        @pl.when(j == 2)
        def _():
            start_mha(0, 14)
            start_mha(0, 15)

        qa_buf[0, j] = project_q(GQA, j)

    lax.fori_loop(0, REP, first_queries, None)

    def gqa_part(m):
        g, pair = m >> 2, m & 3
        slot = g & 1

        @pl.when(pair == 0)
        def _():
            wait_filled(kv_buf.at[2 + slot], a_sem.at[slot])

        def scores(i):
            q = qa_buf[slot, :, _rows(2 * pair + i, SQ)].reshape(REP * SQ, DH)
            return _scores(q, kv_buf[2 + slot, pair, 0, i])

        def attend(i, s):
            o = _weighted(_softmax(s), kv_buf[2 + slot, pair, 1, i])
            return jnp.concatenate([o[j * SQ:(j + 1) * SQ] for j in range(REP)], axis=1)

        start(m, STARTS_IN_GQA_PART[0])
        s0 = scores(0)
        start(m, STARTS_IN_GQA_PART[1])
        qb_buf[m & 1] = project_q(MHA, m)
        start(m, STARTS_IN_GQA_PART[2])
        o0 = attend(0, s0)
        start(m, STARTS_IN_GQA_PART[3])
        s1 = scores(1)
        start(m, STARTS_IN_GQA_PART[4])
        qa_buf[1 - slot, pair] = project_q(GQA, jnp.minimum(m + REP, HQ - 1))
        start(m, STARTS_IN_GQA_PART[5])
        o1 = attend(1, s1)
        start(m, STARTS_IN_GQA_PART[6])
        o = jnp.concatenate([o0, o1], axis=0).astype(jnp.bfloat16)
        w = wo_buf[GQA, g >> 1, _rows(g & 1, REP * DH)]
        acc[GQA, _rows(pair, 2 * SQ)] += jnp.dot(o, w, preferred_element_type=jnp.float32)

    def mha_scores(h, b):
        return _scores(qb_buf[h & 1, _rows(b, SQ)], kv_buf[h & 1, b // 2, 0, b % 2])

    def mha_weighted(h, b, softmax):
        return _weighted(softmax, kv_buf[h & 1, b // 2, 1, b % 2])

    def mha_projected(h, rows, outs):
        o = jnp.concatenate(outs, axis=0).astype(jnp.bfloat16)
        w = wo_buf[MHA, h >> 3, _rows(h & 7, DH)]
        return acc[MHA, rows] + jnp.dot(o, w, preferred_element_type=jnp.float32)

    def mha_part(h):
        wait_filled(kv_buf.at[h & 1], b_sem.at[h & 1])
        s = [mha_scores(h, 0), mha_scores(h, 1)]
        o = []
        for b in range(B):
            start(h + 1, STARTS_IN_MHA_PART[b])
            if b + 2 < B:
                s.append(mha_scores(h, b + 2))
            o.append(mha_weighted(h, b, _softmax(s[b])))
            if b == 5:
                acc[MHA, _rows(0, 4 * SQ)] = mha_projected(h, _rows(0, 4 * SQ), o[0:4])
        acc[MHA, _rows(1, 4 * SQ)] = mha_projected(h, _rows(1, 4 * SQ), o[4:8])

    def step(m, _):
        gqa_part(m)
        pl.when(m > 0)(lambda: mha_part(m - 1))

    lax.fori_loop(0, HQ, step, None)

    h = HQ - 1
    left, right = _rows(GQA, D), _rows(MHA, D)

    def wait_last(pair, kv):
        wait_filled(kv_buf.at[h & 1, pair, kv], b_sem.at[last_sem(pair, kv, 0)])

    def wait_last_v(first, count):
        rows = pl.ds(first * PIECE, count * PIECE)
        wait_filled(kv_buf.at[h & 1, NPAIR - 1, 1, :, rows], b_sem.at[last_sem(NPAIR - 1, 1, first)])

    def finish(pair, outs):
        rows = _rows(pair, 2 * SQ)
        out_buf[rows, right] = mha_projected(h, rows, outs).astype(jnp.bfloat16)

    sends = _output_copies(out_buf, out_hbm, out_sem)
    out_buf[:, left] = acc[GQA].astype(jnp.bfloat16)
    for pair in range(3):
        wait_last(pair, 0)
    wait_last(0, 1)
    s = [mha_scores(h, b) for b in range(3)]
    o0 = mha_weighted(h, 0, _softmax(s[0]))
    s.append(mha_scores(h, 3))
    o1 = mha_weighted(h, 1, _softmax(s[1]))
    s.append(mha_scores(h, 4))
    p2 = _softmax(s[2])
    s.append(mha_scores(h, 5))
    p3 = _softmax(s[3])
    finish(0, [o0, o1])
    p4, p5 = _softmax(s[4]), _softmax(s[5])

    wait_last(1, 1)
    wait_last(3, 0)
    o2, o3 = mha_weighted(h, 2, p2), mha_weighted(h, 3, p3)
    s6, s7 = mha_scores(h, 6), mha_scores(h, 7)
    finish(1, [o2, o3])
    p6, p7 = _softmax(s6), _softmax(s7)

    wait_last(2, 1)
    wait_last_v(0, LAST_SPLIT)
    sends[0].start(priority=0)
    sends[1].start(priority=1)
    finish(2, [mha_weighted(h, 4, p4), mha_weighted(h, 5, p5)])
    sends[2].start(priority=1)

    wait_last_v(LAST_SPLIT, NCHUNK - LAST_SPLIT)
    finish(3, [mha_weighted(h, 6, p6), mha_weighted(h, 7, p7)])
    sends[3].start(priority=0)


@jax.jit
def pallas_concat_heads__gqa_block_cached__mha_block_cached__near_ridge_kernel(
    A_x: jax.Array,
    A_k_cache: jax.Array,
    A_v_cache: jax.Array,
    A_wq: jax.Array,
    A_wo: jax.Array,
    B_x: jax.Array,
    B_k_cache: jax.Array,
    B_v_cache: jax.Array,
    B_wq: jax.Array,
    B_wo: jax.Array,
):
    wq_shape = (WPART, D // WPART, HQ * DH)
    wo_shape = (WPART, HQ * DH // WPART, D)
    kv_shape = (4, NPAIR, 2, 2, SK, DH)
    out = pl.pallas_call(
        _kernel,
        name="gqa_mha_cached_blocks",
        in_specs=[pl.BlockSpec(memory_space=pl.ANY)] * 10,
        out_specs=pl.BlockSpec(memory_space=pl.ANY),
        out_shape=jax.ShapeDtypeStruct((M, 2 * D), jnp.bfloat16),
        scratch_shapes=[
            pltpu.VMEM((2, M, D), jnp.bfloat16),
            pltpu.VMEM((2,) + wq_shape, jnp.bfloat16),
            pltpu.VMEM((2,) + wo_shape, jnp.bfloat16),
            pltpu.VMEM(kv_shape, jnp.bfloat16),
            pltpu.VMEM((2, REP, M, DH), jnp.bfloat16),
            pltpu.VMEM((2, M, DH), jnp.bfloat16),
            pltpu.VMEM((2, M, D), jnp.float32),
            pltpu.VMEM((M, 2 * D), jnp.bfloat16),
            pltpu.SemaphoreType.DMA(()),
        ],
        compiler_params=pltpu.CompilerParams(vmem_limit_bytes=64 * 2**20),
    )(A_x.reshape(M, D), A_k_cache, A_v_cache, A_wq.reshape(wq_shape), A_wo.reshape(wo_shape),
      B_x.reshape(M, D), B_k_cache, B_v_cache, B_wq.reshape(wq_shape), B_wo.reshape(wo_shape))
    return out.reshape(B, SQ, 2 * D)
```
